```python
import os as _os
_os.environ.setdefault("JAX_PLATFORMS", "cpu")
import jax
import jax.numpy as jnp

def _softmax(x, axis=-1):
    return jax.nn.softmax(x, axis=axis)
def _gelu(x):
    return jax.nn.gelu(x, approximate=True)
def _silu(x):
    return jax.nn.silu(x)
def _sigmoid(x):
    return jax.nn.sigmoid(x)
def _layernorm(x, axis=-1, eps=1e-5):
    m = jnp.mean(x, axis=axis, keepdims=True)
    v = jnp.var(x, axis=axis, keepdims=True)
    return (x - m) / jnp.sqrt(v + eps)
def _scatter_add(tgt, idx, src, axis=0):
    return tgt.at[idx].add(src)
def _segment_sum(src, seg, n):
    return jax.ops.segment_sum(src, seg, n)
class _Rng:
    def __init__(self, key):
        self._k = key
    def _next(self):
        self._k, sub = jax.random.split(self._k)
        return sub
    def normal(self, shape):
        return jax.random.normal(self._next(), shape, dtype=jnp.bfloat16)
    def randint(self, lo, hi, shape):
        return jax.random.randint(self._next(), shape, lo, hi, dtype=jnp.int32)
    def uniform(self, shape, lo=0.0, hi=1.0):
        return jax.random.uniform(self._next(), shape, jnp.bfloat16, lo, hi)
    def permutation(self, n):
        return jax.random.permutation(self._next(), n)


kernel_name = 'gated_mix__sliding_local_dilated__moe_arch_mod__prompt'

def setup_inputs():
    _rng = _Rng(jax.random.key(int.from_bytes(__import__("os").urandom(4), "little")))
    _w = (lambda a: (lambda t: t.astype(jnp.bfloat16) if jnp.issubdtype(t.dtype, jnp.floating) else t)(jnp.asarray(a)))
    def _A_setup():
        B, S, D = 1, 2048, 640
        return {
            "x": _w((lambda *s: _rng.normal(s) * 0.05)(B, S, D)),
            "wqkv": _w((lambda *s: _rng.normal(s) * 0.8)(D, 3 * D)),
            "wo": _w((lambda *s: _rng.normal(s) * 0.05)(D, D)),
        }
    _A_in = _A_setup()

    def _B_setup():
        B, S, D, F, C = 1, 2048, 640, 1728, 1
        return {
            "x": _w((lambda *s: _rng.normal(s) * 0.05)(B, S, D)),
            "w_r": _w((lambda *s: _rng.normal(s) * 1.6)(D)),
            "w_gate": _w((lambda *s: _rng.normal(s) * 0.4)(D, F)),
            "w_up": _w((lambda *s: _rng.normal(s) * 0.4)(D, F)),
            "w_down": _w((lambda *s: _rng.normal(s) * 0.4)(F, D)),
        }
    _B_in = _B_setup()

    return {
        "A_x": _A_in["x"],
        "A_wqkv": _A_in["wqkv"],
        "A_wo": _A_in["wo"],
        "B_x": _B_in["x"],
        "B_w_r": _B_in["w_r"],
        "B_w_gate": _B_in["w_gate"],
        "B_w_up": _B_in["w_up"],
        "B_w_down": _B_in["w_down"],
        "gate_w": _w((lambda *s: _rng.normal(s) * 0.05)(640) * 16.0),
    }

def reference(A_x, A_wqkv, A_wo, B_x, B_w_r, B_w_gate, B_w_up, B_w_down, gate_w):
    def _A_ref(x, wqkv, wo):
        B, S, D = x.shape
        H = 32; Dh = D // H
        W, dil = 8, 2
        qkv = (lambda x, *d: x.transpose(*d))((x @ wqkv).reshape(B, S, 3, H, Dh), 2, 0, 3, 1, 4)
        q, k, v = qkv[0], qkv[1], qkv[2]
        scale = Dh ** -0.5
        pos = jnp.arange(S)
        off = jnp.arange(W) * dil
        idx = pos[:, None] - off[None, :]
        mask = idx >= 0
        idx_c = jnp.where(mask, idx, 0).reshape(-1)
        kg = k[:, :, idx_c, :].reshape(B, H, S, W, Dh)
        vg = v[:, :, idx_c, :].reshape(B, H, S, W, Dh)
        logits = jnp.einsum("bhsd,bhswd->bhsw", q, kg) * scale
        logits = jnp.where(mask[None, None, :, :], logits, -1e9)
        attn = _softmax(logits, axis=-1)
        o = jnp.einsum("bhsw,bhswd->bhsd", attn, vg)
        return (lambda x, *d: x.transpose(*d))(o, 0, 2, 1, 3).reshape(B, S, D) @ wo

    def _B_ref(x, w_r, w_gate, w_up, w_down):
        B, S, D = x.shape
        C = 1
        r = x @ w_r
        idx = jnp.argsort(-r, axis=-1)[:, :C]
        idx_e = jnp.repeat(idx.reshape(B, C, 1), D, axis=2)
        x_sel = jnp.take_along_axis(x, idx_e, axis=1)
        g = _silu(x_sel @ w_gate)
        u = x_sel @ w_up
        y = (g * u) @ w_down
        r_sel = _sigmoid(jnp.take_along_axis(r, idx, axis=1))
        y = y * r_sel.reshape(B, C, 1)
        b_off = (jnp.arange(B) * S).reshape(B, 1)
        flat_idx = (idx + b_off).reshape(B * C)
        zero = (x * 0.0).reshape(B * S, D)
        upd = _scatter_add(zero, flat_idx, y.reshape(B * C, D), axis=0)
        return x + upd.reshape(B, S, D)

    x = A_x
    g = _sigmoid((x * gate_w).sum(-1, keepdims=True))
    a = _A_ref(x, A_wqkv, A_wo)
    b = _B_ref(x, B_w_r, B_w_gate, B_w_up, B_w_down)
    return g * a + (1 - g) * b
```

```python
import functools
import jax
import jax.numpy as jnp
import numpy as np
import jax.experimental.pallas as pl
import jax.experimental.pallas.tpu as pltpu

S, D, H, DH, F = 2048, 640, 32, 20, 1728
W, DIL = 8, 2
BM = 128
NB = S // BM
PAD = 16
NT = D // 128
QSCALE = float(DH ** -0.5 * np.log2(np.e))
NEG = float(-1e9 * np.log2(np.e))
CH = 8
ORD = 'ro012a'
FV = 320


def _kernel(x_hbm, wqkv_hbm, wo_hbm, wr_hbm, wg_hbm, wu_hbm, wd_hbm, gw_hbm, o_hbm,
            x_v, wraw_v, woraw_v, wg_v, wu_v, wd_v, wp_v, wop_v, t_v, tf_v,
            qkv_v, o_v, g_v, out_v, sem_x, sem_w, sem_f, sem_o, sem_p, wr_ref, gw_ref):
    f32, bf16 = jnp.float32, jnp.bfloat16

    def x_copy(i, r0, n):
        return pltpu.make_async_copy(x_hbm.at[pl.ds(r0, n)], x_v.at[pl.ds(r0, n)], sem_x.at[i])

    def w_copy(j):
        return pltpu.make_async_copy(wqkv_hbm.at[:, pl.ds(j * D, D)], wraw_v.at[j], sem_w.at[j])

    wo_copy = pltpu.make_async_copy(wo_hbm, woraw_v, sem_w.at[3])
    f_copies = [pltpu.make_async_copy(wg_hbm, wg_v, sem_f.at[0]),
                pltpu.make_async_copy(wu_hbm, wu_v, sem_f.at[1]),
                pltpu.make_async_copy(wd_hbm, wd_v, sem_f.at[2])]

    def o_copy(i, r0, n):
        return pltpu.make_async_copy(out_v.at[pl.ds(r0, n)], o_hbm.at[pl.ds(r0, n)], sem_o.at[i])

    xc = [x_copy(0, 0, 2 * BM), x_copy(1, 2 * BM, 2 * BM), x_copy(2, 4 * BM, S - 4 * BM)]
    KB = ((0, 128), (128, 128), (256, 64))
    wq_copies = [pltpu.make_async_copy(wqkv_hbm.at[pl.ds(2 * k0, 2 * kn), pl.ds(0, D)],
                                       wraw_v.at[0, pl.ds(2 * k0, 2 * kn), :], sem_w.at[4 + kb])
                 for kb, (k0, kn) in enumerate(KB)]
    v_copies = [pltpu.make_async_copy(wr_hbm, wr_ref, sem_w.at[7]), pltpu.make_async_copy(gw_hbm, gw_ref, sem_w.at[8])]
    for c in wq_copies + v_copies:
        c.start()
    xc[0].start()
    w_copy(1).start()

    def perm1(j, kb):
        k0, kn = KB[kb]
        w32 = pltpu.bitcast(wraw_v[j, pl.ds(2 * k0, 2 * kn), :], jnp.uint32)
        t_v[j, kb, :, pl.ds(0, kn)] = w32.T

    def perm2(j, kb):
        k0, kn = KB[kb]
        pm = jnp.concatenate([t_v[j, kb, pl.ds(d, H, stride=DH), :] for d in range(DH)], axis=0)
        wp_v[j, pl.ds(k0, kn), :] = pm[:, :kn].T

    def perm_w(j):
        for kb in range(3):
            perm1(j, kb)
        for kb in range(3):
            perm2(j, kb)

    def perm_wo():
        for t in range(NT):
            tf_v[t] = woraw_v[:, pl.ds(t * 128, 128)].astype(f32)
            for d in range(DH):
                wop_v[pl.ds(d * H // 2, H // 2), pl.ds(t * 128, 128)] = pltpu.bitcast(
                    tf_v[t, pl.ds(d, H, stride=DH), :].astype(bf16), jnp.uint32)

    sub = jax.lax.broadcasted_iota(jnp.int32, (8, 1), 0)

    def al(r):
        return r if isinstance(r, int) else pl.multiple_of(r, BM)

    def proj(r0, n, j):
        y = jnp.dot(x_v[pl.ds(r0, n), :], pltpu.bitcast(wp_v[j], bf16), preferred_element_type=f32)
        if j == 0:
            y = y * QSCALE
        for t in range(NT):
            qkv_v[j * NT + t, pl.ds(r0 + PAD, n), :] = y[:, t * 128:(t + 1) * 128]

    def router(r0, n, top):
        rm, ri = top
        for c in range(n // 16):
            xf = x_v[pl.ds(r0 + c * 16, 16), :].astype(f32)
            g_v[pl.ds(r0 + c * 16, 16), :] = jnp.broadcast_to(
                jax.nn.sigmoid(jnp.sum(xf * gw, axis=-1, keepdims=True)), (16, 128))
            r = jnp.sum(xf * wr, axis=-1, keepdims=True).astype(bf16).astype(f32)
            for h in range(2):
                rr = r[h * 8:(h + 1) * 8]
                gt = rr > rm
                rm = jnp.where(gt, rr, rm)
                ri = jnp.where(gt, sub + (r0 + c * 16 + h * 8), ri)
        return rm, ri

    def att_a(r0):
        qs = [qkv_v[t, pl.ds(r0 + PAD, CH), :] for t in range(NT)]
        P = []
        for w in range(W):
            acc = None
            for t in range(NT):
                p = qs[t] * qkv_v[NT + t, pl.ds(r0 + PAD - DIL * w, CH), :]
                acc = p if acc is None else acc + p
            P.append((acc, pltpu.roll(acc, 64, 1)))
        return P

    def att_b(P):
        out = []
        for a, b in P:
            c = a + b
            out.append((c, pltpu.roll(c, 32, 1)))
        return out

    def att_c(r0, P):
        L = [a + b for a, b in P]
        if isinstance(r0, int) and r0 < DIL * (W - 1):
            pos = r0 + jax.lax.broadcasted_iota(jnp.int32, (CH, 128), 0)
            L = [jnp.where(pos >= DIL * w, L[w], NEG) if DIL * w > r0 else L[w] for w in range(W)]
        m = functools.reduce(jnp.maximum, L)
        e = [jnp.exp2(l - m) for l in L]
        ssum = functools.reduce(jnp.add, e)
        inv = pl.reciprocal(ssum, approx=True)
        inv = inv * (2.0 - ssum * inv)
        outs = []
        for t in range(NT):
            acc = None
            for w in range(W):
                p = e[w] * qkv_v[2 * NT + t, pl.ds(r0 + PAD - DIL * w, CH), :]
                acc = p if acc is None else acc + p
            outs.append(acc * inv)
        return outs

    def attn(lo, n):
        st, res = {}, {}
        n = n // CH
        for c in range(n + 2):
            if c >= 2:
                cc = c - 2
                res[cc] = att_c(lo + cc * CH, st.pop(cc))
                if cc % 2 == 1:
                    for t in range(NT):
                        o_v[pl.ds(lo + (cc - 1) * CH, 2 * CH), pl.ds(t * 128, 128)] = jnp.concatenate(
                            [res[cc - 1][t], res[cc][t]], axis=0).astype(bf16)
            if 0 <= c - 1 < n:
                st[c - 1] = att_b(st[c - 1])
            if c < n:
                st[c] = att_a(lo + c * CH)

    def outp(r0, n):
        a = jnp.dot(o_v[pl.ds(r0, n), :], pltpu.bitcast(wop_v[...], bf16), preferred_element_type=f32)
        g = g_v[pl.ds(r0, n), :]
        for t in range(NT):
            xf = x_v[pl.ds(r0, n), pl.ds(t * 128, 128)].astype(f32)
            out_v[pl.ds(r0, n), pl.ds(t * 128, 128)] = (xf + g * (a[:, t * 128:(t + 1) * 128] - xf)).astype(bf16)

    wq_copies[0].wait()
    perm1(0, 0)
    wq_copies[1].wait()
    wq_copies[2].wait()
    w_copy(2).start()
    perm1(0, 1)
    perm1(0, 2)
    for kb in range(3):
        perm2(0, kb)
    for c in v_copies:
        c.wait()
    xc[0].wait()
    gw = gw_ref[...].astype(f32).reshape(1, D)
    wr = wr_ref[...].astype(f32).reshape(1, D)
    proj(0, BM, 0)
    top = router(0, BM, (jnp.full((8, 1), -jnp.inf, f32), sub))
    w_copy(1).wait()
    xc[1].start()
    wo_copy.start()
    proj(BM, BM, 0)
    perm_w(1)
    w_copy(2).wait()
    proj(0, 2 * BM, 1)
    perm_w(2)
    top = router(BM, BM, top)
    xc[1].wait()
    wo_copy.wait()
    xc[2].start()
    proj(0, BM, 2)
    proj(BM, BM, 2)
    for t in range(NT):
        for j in (1, 2):
            qkv_v[j * NT + t, pl.ds(0, PAD), :] = jnp.broadcast_to(qkv_v[j * NT + t, pl.ds(PAD, 1), :], (PAD, 128))
    attn(0, BM)
    perm_wo()

    def body(i, top):
        prev, cur, nxt = al((i - 1) * BM), al(i * BM), al((i + 1) * BM)
        for ch in ORD:
            if ch == 'o':
                outp(prev, BM)
            elif ch == 'r':
                top = router(nxt, BM, top)
            elif ch == 'a':
                attn(cur, BM)
            else:
                proj(nxt, BM, int(ch))
        o_copy(i - 1, prev, BM).start()

        @pl.when(i == 2)
        def _():
            xc[2].wait()
            for c in f_copies:
                c.start()
        return top
    rm, ri = jax.lax.fori_loop(1, NB - 1, body, top)
    f_copies[0].wait()
    f_copies[1].wait()
    f_copies[2].wait()
    for i in range(NB - 3):
        o_copy(i, i * BM, BM).wait()

    rmax = jnp.max(rm)
    idx = jnp.min(jnp.where(rm == rmax, ri, S - 1))
    pb = pl.multiple_of((idx // 16) * 16, 16)
    xt = x_v[pl.ds(pb, 16), :]
    FM = F - FV
    outp((NB - 2) * BM, BM)
    nt_dims = (((1,), (1,)), ((), ()))
    hg = jax.lax.dot_general(xt, wg_v[pl.ds(0, FM), :], nt_dims, preferred_element_type=f32)
    hu = jax.lax.dot_general(xt, wu_v[pl.ds(0, FM), :], nt_dims, preferred_element_type=f32)
    attn((NB - 1) * BM, BM)
    outp((NB - 1) * BM, BM)
    hh = (hg * jax.nn.sigmoid(hg) * hu).astype(bf16)
    y = jnp.dot(hh, wd_v[pl.ds(0, FM), :], preferred_element_type=f32)
    sel = jax.lax.broadcasted_iota(jnp.int32, (16, D), 0) == idx - pb
    if FV:
        xs = jnp.sum(jnp.where(sel, xt.astype(f32), 0.0), axis=0, keepdims=True)
        acc = jnp.zeros((16, D), f32)
        for c in range(FV // 16):
            rows = pl.ds(FM + c * 16, 16)
            vg = jnp.sum(wg_v[rows, :].astype(f32) * xs, axis=-1, keepdims=True)
            vu = jnp.sum(wu_v[rows, :].astype(f32) * xs, axis=-1, keepdims=True)
            acc = acc + (vg * jax.nn.sigmoid(vg) * vu) * wd_v[rows, :].astype(f32)
        y = y + jnp.sum(acc, axis=0, keepdims=True)
    g = g_v[pl.ds(pb, 16), :][:, 0:1]
    y = y * jax.nn.sigmoid(jnp.full((16, 1), rmax, f32)) * (1.0 - g)
    o_copy(NB - 3, (NB - 3) * BM, BM).wait()
    cur = out_v[pl.ds(pb, 16), :].astype(f32)
    out_v[pl.ds(pb, 16), :] = jnp.where(sel, cur + y, cur).astype(bf16)
    last = o_copy(NB - 2, (NB - 2) * BM, 2 * BM)
    last.start()

    @pl.when(pb < (NB - 2) * BM)
    def _():
        pc = pltpu.make_async_copy(out_v.at[pl.ds(pb, 16)], o_hbm.at[pl.ds(pb, 16)], sem_p)
        pc.start()
        pc.wait()
    last.wait()


@jax.jit
def pallas_gated_mix__sliding_local_dilated__moe_arch_mod__prompt_kernel(A_x, A_wqkv, A_wo, B_x, B_w_r, B_w_gate, B_w_up, B_w_down, gate_w):
    f32, bf16 = jnp.float32, jnp.bfloat16
    anyspec = pl.BlockSpec(memory_space=pltpu.HBM)
    out = pl.pallas_call(
        _kernel,
        out_shape=jax.ShapeDtypeStruct((S, D), bf16),
        in_specs=[anyspec] * 8,
        out_specs=anyspec,
        scratch_shapes=[
            pltpu.VMEM((S, D), bf16),
            pltpu.VMEM((3, D, D), bf16),
            pltpu.VMEM((D, D), bf16),
            pltpu.VMEM((F, D), bf16), pltpu.VMEM((F, D), bf16), pltpu.VMEM((F, D), bf16),
            pltpu.VMEM((3, D // 2, D), jnp.uint32),
            pltpu.VMEM((D // 2, D), jnp.uint32),
            pltpu.VMEM((3, 3, D, 128), jnp.uint32),
            pltpu.VMEM((NT, D, 128), f32),
            pltpu.VMEM((3 * NT, S + PAD, 128), f32),
            pltpu.VMEM((S, D), bf16),
            pltpu.VMEM((S, 128), f32),
            pltpu.VMEM((S, D), bf16),
            pltpu.SemaphoreType.DMA((3,)), pltpu.SemaphoreType.DMA((9,)),
            pltpu.SemaphoreType.DMA((3,)), pltpu.SemaphoreType.DMA((NB,)),
            pltpu.SemaphoreType.DMA(()),
            pltpu.VMEM((D,), bf16), pltpu.VMEM((D,), bf16),
        ],
        compiler_params=pltpu.CompilerParams(vmem_limit_bytes=100 * 1024 * 1024),
    )(A_x.reshape(S, D), A_wqkv, A_wo, B_w_r, B_w_gate.T, B_w_up.T, B_w_down, gate_w)
    return out.reshape(1, S, D)
```
